```python
import jax
import jax.numpy as jnp

def _softmax(x, axis=-1):
    return jax.nn.softmax(x, axis=axis)
def _gelu(x):
    return jax.nn.gelu(x, approximate=True)
def _silu(x):
    return jax.nn.silu(x)
def _sigmoid(x):
    return jax.nn.sigmoid(x)
def _layernorm(x, axis=-1, eps=1e-5):
    m = jnp.mean(x, axis=axis, keepdims=True)
    v = jnp.var(x, axis=axis, keepdims=True)
    return (x - m) / jnp.sqrt(v + eps)
def _scatter_add(tgt, idx, src, axis=0):
    return tgt.at[idx].add(src)
def _segment_sum(src, seg, n):
    return jax.ops.segment_sum(src, seg, n)
class _Rng:
    def __init__(self, key):
        self._k = key
    def _next(self):
        self._k, sub = jax.random.split(self._k)
        return sub
    def normal(self, shape):
        return jax.random.normal(self._next(), shape, dtype=jnp.bfloat16)
    def randint(self, lo, hi, shape):
        return jax.random.randint(self._next(), shape, lo, hi, dtype=jnp.int32)
    def uniform(self, shape, lo=0.0, hi=1.0):
        return jax.random.uniform(self._next(), shape, jnp.bfloat16, lo, hi)
    def permutation(self, n):
        return jax.random.permutation(self._next(), n)


kernel_name = 'standalone__structured_sparse_n_m__ragged'

def setup_inputs():
    _rng = _Rng(jax.random.key(int.from_bytes(__import__("os").urandom(4), "little")))
    _w = (lambda a: (lambda t: t.astype(jnp.bfloat16) if jnp.issubdtype(t.dtype, jnp.floating) else t)(jnp.asarray(a)))
    B, S, D = 16, 4096, 576
    assert D % 4 == 0, "d_model must be divisible by M=4 for 2:4 sparsity"
    return {
        "x": _w((lambda *s: _rng.normal(s) * 0.05)(B, S, D)),
        "w": _w((lambda *s: _rng.normal(s) * 0.05)(D, D)),
        "b": _w((lambda *s: _rng.normal(s) * 0.05)(D)),
    }

def reference(x, w, b):
    B, S, D = x.shape
    N, M = 2, 4
    G = D // M
    wg = w.reshape(G, M, D)
    mag = jnp.abs(wg)
    order = jnp.argsort(mag, 1)
    thr = jnp.take_along_axis(mag, order[:, M - N:M - N + 1, :], 1)
    mask = (lambda x, dt: x.astype(dt))(mag >= thr, w.dtype)
    wp = (wg * mask).reshape(D, D)
    return jnp.einsum("bsd,df->bsf", x, wp) + b
```

```python
import jax
import jax.numpy as jnp
from jax import lax
import jax.experimental.pallas as pl
import jax.experimental.pallas.tpu as pltpu

KA = 16
HEAD = (512, 1024, 2560)
NREP = 2
NB = 2
OSPLIT = ((4096,), (2048, 1024, 512, 256, 128, 128))
NX, NO = 4, 4


def _prune_2_4(w):
    R, C = w.shape
    u = pltpu.bitcast(w, jnp.uint32).reshape(R // 16, 8, C)
    a = pltpu.bitcast((u << 16) & jnp.uint32(0x7FFF0000), jnp.float32)
    b = pltpu.bitcast(u & jnp.uint32(0x7FFF0000), jnp.float32)
    mx, mn = jnp.maximum(a, b), jnp.minimum(a, b)
    mx1, mn1 = pltpu.roll(mx, 7, 1), pltpu.roll(mn, 7, 1)
    thr = jnp.maximum(jnp.minimum(mx, mx1), jnp.maximum(mn, mn1))
    sub = lax.broadcasted_iota(jnp.int32, u.shape, 1)
    thr = jnp.where((sub & 1) == 0, thr, pltpu.roll(thr, 1, 1))
    keep = (jnp.where(a >= thr, jnp.uint32(0x0000FFFF), jnp.uint32(0))
            | jnp.where(b >= thr, jnp.uint32(0xFFFF0000), jnp.uint32(0)))
    return pltpu.bitcast((u & keep).reshape(R // 2, C), jnp.bfloat16)


def _kernel(x_hbm, w_hbm, b_hbm, o_hbm, xbuf, obuf, wbuf, bbuf, wt_ref, xsem, osem, wsem, hsem):
    B, D, S = x_hbm.shape
    nh = len(HEAD)
    offs = [sum(HEAD[:i]) for i in range(nh)]

    def mm(xs, os_, lo, n):
        row = lax.broadcasted_iota(jnp.int32, (KA, n), 0)
        ones = jnp.where(row == 0, 1.0, 0.0).astype(jnp.bfloat16)
        xa = jnp.concatenate([xbuf[xs, :, pl.ds(lo, n)], ones], axis=0)
        acc = jnp.dot(wt_ref[...], xa, preferred_element_type=jnp.float32)
        obuf[os_, :, pl.ds(lo, n)] = acc.astype(obuf.dtype)

    def xcp(bi, slot):
        return pltpu.make_async_copy(x_hbm.at[bi], xbuf.at[slot], xsem.at[slot])

    def opiece(bi, slot, lo, n):
        return pltpu.make_async_copy(obuf.at[slot, :, pl.ds(lo, n)], o_hbm.at[bi, :, pl.ds(lo, n)], osem.at[slot])

    def owait(bi, slot):
        pltpu.make_async_copy(obuf.at[slot], o_hbm.at[bi], osem.at[slot]).wait()

    def hcp(r, i):
        return pltpu.make_async_copy(x_hbm.at[r, :, pl.ds(offs[i], HEAD[i])],
                                     xbuf.at[r, :, pl.ds(offs[i], HEAD[i])], hsem.at[r * nh + i])

    w_cp = pltpu.make_async_copy(w_hbm, wbuf, wsem.at[0])
    b_cp = pltpu.make_async_copy(b_hbm, bbuf, wsem.at[1])
    w_cp.start()
    b_cp.start()
    hcp(0, 0).start()
    w_cp.wait()
    b_cp.wait()
    for r in range(NREP):
        for i in range(nh):
            if (r, i) != (0, 0):
                hcp(r, i).start()
    for bi in range(NREP, min(NX, B)):
        xcp(bi, bi).start()

    wp = _prune_2_4(wbuf[...])
    row = lax.broadcasted_iota(jnp.int32, (KA, D), 0)
    brow = jnp.where(row == 0, jnp.broadcast_to(bbuf[...].astype(jnp.float32).reshape(1, D), (KA, D)), 0.0)
    wt_ref[...] = jnp.concatenate([wp, brow.astype(jnp.bfloat16)], axis=0).T

    def rep(r, c):
        for i in range(nh):
            hcp(r, i).wait()
            if i == nh - 1:
                @pl.when(r > 0)
                def _():
                    opiece(r - 1, r - 1, 0, S).start()
            mm(r, r, offs[i], HEAD[i])
        return c

    lax.fori_loop(0, NREP, rep, 0)
    opiece(NREP - 1, NREP - 1, 0, S).start()
    for bi in range(NX, min(NX + NREP - NB, B)):
        xcp(bi, bi % NX).start()

    def body(t, c):
        b0 = NREP + t * NB
        for j in range(NB):
            nxt = b0 + j - NB + NX

            @pl.when(nxt < B)
            def _():
                xcp(nxt, nxt % NX).start()
        for j in range(NB):
            xcp(b0 + j, (b0 + j) % NX).wait()
        for j in range(NB):
            @pl.when(b0 + j >= NO)
            def _():
                owait(b0 + j - NO, (b0 + j) % NO)
        for j in range(NB):
            bi = b0 + j
            lo = 0
            for n in OSPLIT[j]:
                mm(bi % NX, bi % NO, lo, n)
                opiece(bi, bi % NO, lo, n).start()
                lo += n
        return c

    lax.fori_loop(0, (B - NREP) // NB, body, 0)
    for bi in range(max(B - NO, 0), B):
        owait(bi, bi % NO)


@jax.jit
def pallas_standalone__structured_sparse_n_m__ragged_kernel(
    x: jax.Array,
    w: jax.Array,
    b: jax.Array,
):
    B, S, D = x.shape
    xt = jnp.transpose(x, (0, 2, 1))
    hbm = pl.BlockSpec(memory_space=pltpu.HBM)
    out = pl.pallas_call(
        _kernel,
        in_specs=[hbm, hbm, hbm],
        out_specs=hbm,
        out_shape=jax.ShapeDtypeStruct((B, D, S), x.dtype),
        scratch_shapes=[
            pltpu.VMEM((NX, D, S), jnp.bfloat16),
            pltpu.VMEM((NO, D, S), jnp.bfloat16),
            pltpu.VMEM((D, D), jnp.bfloat16),
            pltpu.VMEM((D,), jnp.bfloat16),
            pltpu.VMEM((D, D + KA), jnp.bfloat16),
            pltpu.SemaphoreType.DMA((NX,)),
            pltpu.SemaphoreType.DMA((NO,)),
            pltpu.SemaphoreType.DMA((2,)),
            pltpu.SemaphoreType.DMA((NREP * len(HEAD),)),
        ],
        compiler_params=pltpu.CompilerParams(vmem_limit_bytes=120 << 20),
    )(xt, w, b)
    return jnp.transpose(out, (0, 2, 1))
```

```python
import jax
import jax.numpy as jnp
from jax import lax
import jax.experimental.pallas as pl
import jax.experimental.pallas.tpu as pltpu

LANES = 128
KA = 16
HEAD = (512, 1024, 2560)
NREP = 2
NB = 2
OSPLIT = ((2048, 2048), (2048, 1024, 512, 256, 256))
NX, NO = 4, 4
GS = 16
VG = (4, 13, 22, 31)
CB, DN = 128, 512


def _prune_2_4(w):
    R, C = w.shape
    u = pltpu.bitcast(w, jnp.uint32).reshape(R // 16, 8, C)
    a = pltpu.bitcast((u << 16) & jnp.uint32(0x7FFF0000), jnp.float32)
    b = pltpu.bitcast(u & jnp.uint32(0x7FFF0000), jnp.float32)
    mx, mn = jnp.maximum(a, b), jnp.minimum(a, b)
    mx1, mn1 = pltpu.roll(mx, 7, 1), pltpu.roll(mn, 7, 1)
    thr = jnp.maximum(jnp.minimum(mx, mx1), jnp.maximum(mn, mn1))
    sub = lax.broadcasted_iota(jnp.int32, u.shape, 1)
    thr = jnp.where((sub & 1) == 0, thr, pltpu.roll(thr, 1, 1))
    keep = (jnp.where(a >= thr, jnp.uint32(0x0000FFFF), jnp.uint32(0))
            | jnp.where(b >= thr, jnp.uint32(0xFFFF0000), jnp.uint32(0)))
    return pltpu.bitcast((u & keep).reshape(R // 2, C), jnp.bfloat16)


def _kernel(x_hbm, w_hbm, b_hbm, o_hbm, xbuf, obuf, wbuf, bbuf, wt_ref, wr_ref, wv_ref, wb_ref, bv_ref, xf_ref,
            xsem, osem, wsem, hsem):
    B, D, S = x_hbm.shape
    nh = len(HEAD)
    offs = [sum(HEAD[:i]) for i in range(nh)]
    K0 = D // LANES * LANES
    KT = D - K0
    NG = D // GS
    MG = [g for g in range(NG) if g not in VG]
    F = GS * len(VG)

    def ones_aug(xs, lo, n, k0):
        row = lax.broadcasted_iota(jnp.int32, (KA, n), 0)
        ones = jnp.where(row == 0, 1.0, 0.0).astype(jnp.bfloat16)
        return jnp.concatenate([xbuf[xs, k0:, pl.ds(lo, n)], ones], axis=0)

    def mm(xs, os_, lo, n):
        acc = jnp.dot(wt_ref[...], ones_aug(xs, lo, n, 0), preferred_element_type=jnp.float32)
        obuf[os_, :, pl.ds(lo, n)] = acc.astype(obuf.dtype)

    cnt = [0]

    def vtail(xs, c):
        xf = xf_ref.at[cnt[0] % xf_ref.shape[0]]
        cnt[0] += 1
        xf[...] = xbuf[xs, K0:D, pl.ds(c, CB)].astype(jnp.float32)
        res = {}
        for i, g in enumerate(VG):
            acc = jnp.concatenate([bv_ref[i * GS:(i + 1) * GS, :]] * (CB // LANES), axis=1)
            for k in range(KT):
                kb, r = divmod(k, 8)
                xr = xf[8 * kb:8 * kb + 8, :]
                if r:
                    xr = pltpu.roll(xr, 8 - r, 0)
                xr = jnp.concatenate([xr] * (GS // 8), axis=0)
                wk = jnp.concatenate([wb_ref[k, i * GS:(i + 1) * GS, :]] * (CB // LANES), axis=1)
                acc = acc + wk * xr
            res[g] = acc
        return res

    def mm_split(xs, os_, lo, n):
        d = min(DN, n)
        for c0 in range(lo, lo + n, d):
            vs = [vtail(xs, c) for c in range(c0, c0 + d, CB)]
            main = jnp.dot(wt_ref[:, :K0], xbuf[xs, :K0, pl.ds(c0, d)], preferred_element_type=jnp.float32)
            rem = jnp.dot(wr_ref[...], ones_aug(xs, c0, d, K0), preferred_element_type=jnp.float32)
            for g in range(NG):
                m = main[g * GS:(g + 1) * GS]
                if g in VG:
                    t = jnp.concatenate([v[g] for v in vs], axis=1)
                else:
                    j = MG.index(g)
                    t = rem[j * GS:(j + 1) * GS]
                obuf[os_, g * GS:(g + 1) * GS, pl.ds(c0, d)] = (m + t).astype(obuf.dtype)

    def build_wb():
        wv = wv_ref[...]
        for k in range(KT):
            wb_ref[k] = jnp.broadcast_to(wv[:, k:k + 1], (F, LANES))

    def xcp(bi, slot):
        return pltpu.make_async_copy(x_hbm.at[bi], xbuf.at[slot], xsem.at[slot])

    def opiece(bi, slot, lo, n):
        return pltpu.make_async_copy(obuf.at[slot, :, pl.ds(lo, n)], o_hbm.at[bi, :, pl.ds(lo, n)], osem.at[slot])

    def owait(bi, slot):
        pltpu.make_async_copy(obuf.at[slot], o_hbm.at[bi], osem.at[slot]).wait()

    def hcp(r, i):
        return pltpu.make_async_copy(x_hbm.at[r, :, pl.ds(offs[i], HEAD[i])],
                                     xbuf.at[r, :, pl.ds(offs[i], HEAD[i])], hsem.at[r * nh + i])

    w_cp = pltpu.make_async_copy(w_hbm, wbuf, wsem.at[0])
    b_cp = pltpu.make_async_copy(b_hbm, bbuf, wsem.at[1])
    w_cp.start()
    b_cp.start()
    hcp(0, 0).start()
    w_cp.wait()
    b_cp.wait()
    for r in range(NREP):
        for i in range(nh):
            if (r, i) != (0, 0):
                hcp(r, i).start()
    for bi in range(NREP, min(NX, B)):
        xcp(bi, bi).start()

    wp = _prune_2_4(wbuf[...])
    row = lax.broadcasted_iota(jnp.int32, (KA, D), 0)
    brow = jnp.where(row == 0, jnp.broadcast_to(bbuf[...].astype(jnp.float32).reshape(1, D), (KA, D)), 0.0)
    wt = jnp.concatenate([wp, brow.astype(jnp.bfloat16)], axis=0).T
    wt_ref[...] = wt
    wtail = wt[:, K0:]
    wr_ref[...] = jnp.concatenate([wtail[g * GS:(g + 1) * GS] for g in MG], axis=0)
    t = wp[K0:].astype(jnp.float32).reshape(KT // 8, 8, D)
    lane = lax.broadcasted_iota(jnp.int32, t.shape, 2)
    for bit in (1, 2, 4):
        t = jnp.where((lane & bit) != 0, pltpu.roll(t, 8 - bit, 1), t)
    tT = jnp.concatenate([t.reshape(KT, D), jnp.zeros((LANES - KT, D), jnp.float32)], axis=0).T
    wv_ref[...] = jnp.concatenate([tT[g * GS:(g + 1) * GS] for g in VG], axis=0)
    bcol = wtail.astype(jnp.float32)[:, KT:KT + 1]
    bv_ref[...] = jnp.broadcast_to(jnp.concatenate([bcol[g * GS:(g + 1) * GS] for g in VG], axis=0), (F, LANES))

    def rep(r, c):
        for i in range(nh):
            hcp(r, i).wait()
            if i == nh - 1:
                @pl.when(r > 0)
                def _():
                    opiece(r - 1, r - 1, 0, S).start()
                build_wb()
            mm(r, r, offs[i], HEAD[i])
        return c

    lax.fori_loop(0, NREP, rep, 0)
    opiece(NREP - 1, NREP - 1, 0, S).start()
    for bi in range(NX, min(NX + NREP - NB, B)):
        xcp(bi, bi % NX).start()

    def body(t, c):
        b0 = NREP + t * NB
        for j in range(NB):
            nxt = b0 + j - NB + NX

            @pl.when(nxt < B)
            def _():
                xcp(nxt, nxt % NX).start()
        for j in range(NB):
            xcp(b0 + j, (b0 + j) % NX).wait()
        for j in range(NB):
            @pl.when(b0 + j >= NO)
            def _():
                owait(b0 + j - NO, (b0 + j) % NO)
        for j in range(NB):
            bi = b0 + j
            lo = 0
            for n in OSPLIT[j]:
                mm_split(bi % NX, bi % NO, lo, n)
                opiece(bi, bi % NO, lo, n).start()
                lo += n
        return c

    lax.fori_loop(0, (B - NREP) // NB, body, 0)
    for bi in range(max(B - NO, 0), B):
        owait(bi, bi % NO)


@jax.jit
def pallas_standalone__structured_sparse_n_m__ragged_kernel(
    x: jax.Array,
    w: jax.Array,
    b: jax.Array,
):
    B, S, D = x.shape
    F = GS * len(VG)
    KT = D - D // LANES * LANES
    xt = jnp.transpose(x, (0, 2, 1))
    hbm = pl.BlockSpec(memory_space=pltpu.HBM)
    out = pl.pallas_call(
        _kernel,
        in_specs=[hbm, hbm, hbm],
        out_specs=hbm,
        out_shape=jax.ShapeDtypeStruct((B, D, S), x.dtype),
        scratch_shapes=[
            pltpu.VMEM((NX, D, S), jnp.bfloat16),
            pltpu.VMEM((NO, D, S), jnp.bfloat16),
            pltpu.VMEM((D, D), jnp.bfloat16),
            pltpu.VMEM((D,), jnp.bfloat16),
            pltpu.VMEM((D, D + KA), jnp.bfloat16),
            pltpu.VMEM((D - F, KT + KA), jnp.bfloat16),
            pltpu.VMEM((F, LANES), jnp.float32),
            pltpu.VMEM((KT, F, LANES), jnp.float32),
            pltpu.VMEM((F, LANES), jnp.float32),
            pltpu.VMEM((4, KT, CB), jnp.float32),
            pltpu.SemaphoreType.DMA((NX,)),
            pltpu.SemaphoreType.DMA((NO,)),
            pltpu.SemaphoreType.DMA((2,)),
            pltpu.SemaphoreType.DMA((NREP * len(HEAD),)),
        ],
        compiler_params=pltpu.CompilerParams(vmem_limit_bytes=120 << 20),
    )(xt, w, b)
    return jnp.transpose(out, (0, 2, 1))
```

```python
import jax
import jax.numpy as jnp
from jax import lax
import jax.experimental.pallas as pl
import jax.experimental.pallas.tpu as pltpu

LANES = 128
KA = 16
HEAD = (512, 1024, 2560)
OSPLIT = ((4096,), (2048, 1024, 512, 256, 128, 128))
GS = 16
VG = (1, 10, 20, 30)
HVG = (1, 10, 30)
DN = 512
XFS = 4


def _prune_2_4(w):
    R, C = w.shape
    u = pltpu.bitcast(w, jnp.uint32).reshape(R // 16, 8, C)
    a = pltpu.bitcast((u << 16) & jnp.uint32(0x7FFF0000), jnp.float32)
    b = pltpu.bitcast(u & jnp.uint32(0x7FFF0000), jnp.float32)
    mx, mn = jnp.maximum(a, b), jnp.minimum(a, b)
    mx1, mn1 = pltpu.roll(mx, 7, 1), pltpu.roll(mn, 7, 1)
    thr = jnp.maximum(jnp.minimum(mx, mx1), jnp.maximum(mn, mn1))
    sub = lax.broadcasted_iota(jnp.int32, u.shape, 1)
    thr = jnp.where((sub & 1) == 0, thr, pltpu.roll(thr, 1, 1))
    keep = (jnp.where(a >= thr, jnp.uint32(0x0000FFFF), jnp.uint32(0))
            | jnp.where(b >= thr, jnp.uint32(0xFFFF0000), jnp.uint32(0)))
    return pltpu.bitcast((u & keep).reshape(R // 2, C), jnp.bfloat16)


def _kernel(x_hbm, w_hbm, b_hbm, o_hbm, xbuf, obuf, wbuf, bbuf, wt_ref, wp_ref, wr_ref, wh_ref,
            wv_ref, wb_ref, bv_ref, xf_ref, xsem, osem, wsem, hsem):
    B, D, S = x_hbm.shape
    NP = B // 2
    nh = len(HEAD)
    offs = [sum(HEAD[:i]) for i in range(nh)]
    K0 = D // LANES * LANES
    KT = D - K0
    NG = D // GS
    F = GS * len(VG)

    def ldw(ref, k):
        return pltpu.bitcast(ref[:, :k], jnp.bfloat16)

    def stw(ref, v):
        ref[...] = pltpu.bitcast(v, jnp.uint32)

    def rows(a, groups):
        return jnp.concatenate([a[g * GS:(g + 1) * GS] for g in groups], axis=0)

    def x_ones(s, j, k0, lo, n):
        row = lax.broadcasted_iota(jnp.int32, (KA, n), 0)
        ones = jnp.where(row == 0, 1.0, 0.0).astype(jnp.bfloat16)
        return jnp.concatenate([xbuf[s, j, k0:, pl.ds(lo, n)], ones], axis=0)

    def mm_dense(s, j, lo, n):
        acc = jnp.dot(ldw(wt_ref, D + KA), x_ones(s, j, 0, lo, n), preferred_element_type=jnp.float32)
        obuf[s, j, :, pl.ds(lo, n)] = acc.astype(obuf.dtype)

    cnt = [0]

    def vpu_tail(s, j, c, groups):
        xf = xf_ref.at[cnt[0] % XFS]
        cnt[0] += 1
        xf[...] = xbuf[s, j, K0:D, pl.ds(c, LANES)].astype(jnp.float32)
        res = {}
        for g in groups:
            i = VG.index(g)
            acc = bv_ref[i * GS:(i + 1) * GS, :]
            for k in range(KT):
                kb, r = divmod(k, 8)
                xr = xf[8 * kb:8 * kb + 8, :]
                if r:
                    xr = pltpu.roll(xr, 8 - r, 0)
                xr = jnp.concatenate([xr] * (GS // 8), axis=0)
                acc = acc + wb_ref[k, i * GS:(i + 1) * GS, :] * xr
            res[g] = acc
        return res

    def mm_split(s, j, lo, n, groups, wrem_ref, hook=None):
        d = min(DN, n)
        mxu_groups = [g for g in range(NG) if g not in groups]
        for c0 in range(lo, lo + n, d):
            vs = [vpu_tail(s, j, c, groups) for c in range(c0, c0 + d, LANES)]
            main = jnp.dot(ldw(wt_ref, K0), xbuf[s, j, :K0, pl.ds(c0, d)], preferred_element_type=jnp.float32)
            rem = jnp.dot(ldw(wrem_ref, KT + KA), x_ones(s, j, K0, c0, d), preferred_element_type=jnp.float32)
            for g in range(NG):
                if g in groups:
                    t = jnp.concatenate([v[g] for v in vs], axis=1)
                else:
                    q = mxu_groups.index(g)
                    t = rem[q * GS:(q + 1) * GS]
                obuf[s, j, g * GS:(g + 1) * GS, pl.ds(c0, d)] = (main[g * GS:(g + 1) * GS] + t).astype(obuf.dtype)
            if c0 == lo and hook is not None:
                hook()

    def prep_tail_tables():
        wtail = ldw(wt_ref, D + KA)[:, K0:]
        stw(wr_ref, rows(wtail, [g for g in range(NG) if g not in VG]))
        stw(wh_ref, rows(wtail, [g for g in range(NG) if g not in HVG]))
        t = pltpu.bitcast(wp_ref[...], jnp.bfloat16).astype(jnp.float32).reshape(KT // 8, 8, D)
        lane = lax.broadcasted_iota(jnp.int32, t.shape, 2)
        for bit in (1, 2, 4):
            t = jnp.where((lane & bit) != 0, pltpu.roll(t, 8 - bit, 1), t)
        tT = jnp.concatenate([t.reshape(KT, D), jnp.zeros((LANES - KT, D), jnp.float32)], axis=0).T
        wv = rows(tT, VG)
        bv_ref[...] = jnp.broadcast_to(rows(wtail.astype(jnp.float32)[:, KT:KT + 1], VG), (F, LANES))
        for k in range(KT):
            wb_ref[k] = jnp.broadcast_to(wv[:, k:k + 1], (F, LANES))

    def xcp(p, s):
        return pltpu.make_async_copy(x_hbm.at[pl.ds(2 * p, 2)], xbuf.at[s], xsem.at[s])

    def opiece(p, s, j, lo, n):
        return pltpu.make_async_copy(obuf.at[s, j, :, pl.ds(lo, n)], o_hbm.at[2 * p + j, :, pl.ds(lo, n)],
                                     osem.at[s])

    def owait(p, s):
        pltpu.make_async_copy(obuf.at[s], o_hbm.at[pl.ds(2 * p, 2)], osem.at[s]).wait()

    def hcp(r, i):
        return pltpu.make_async_copy(x_hbm.at[r, :, pl.ds(offs[i], HEAD[i])],
                                     xbuf.at[0, r, :, pl.ds(offs[i], HEAD[i])], hsem.at[r * nh + i])

    w_cp = pltpu.make_async_copy(w_hbm, wbuf, wsem.at[0])
    b_cp = pltpu.make_async_copy(b_hbm, bbuf, wsem.at[1])
    w_cp.start()
    b_cp.start()
    hcp(0, 0).start()
    w_cp.wait()
    b_cp.wait()
    for r in range(2):
        for i in range(nh):
            if (r, i) != (0, 0):
                hcp(r, i).start()
    xcp(1, 1).start()

    wp = _prune_2_4(wbuf[...])
    row = lax.broadcasted_iota(jnp.int32, (KA, D), 0)
    brow = jnp.where(row == 0, jnp.broadcast_to(bbuf[...].astype(jnp.float32).reshape(1, D), (KA, D)), 0.0)
    stw(wt_ref, jnp.concatenate([wp, brow.astype(jnp.bfloat16)], axis=0).T)
    stw(wp_ref, wp[K0:])

    def head(r, c):
        def start_first_out():
            @pl.when(r > 0)
            def _():
                opiece(0, 0, 0, 0, S).start()

        hcp(r, 0).wait()
        prep_tail_tables()
        mm_dense(0, r, offs[0], HEAD[0])
        for i in range(1, nh):
            hcp(r, i).wait()
            mm_split(0, r, offs[i], HEAD[i], HVG, wh_ref, start_first_out if i == nh - 1 else None)
        return c

    lax.fori_loop(0, 2, head, 0)
    xcp(2, 0).start()

    def body(p, c):
        s = p % 2
        xcp(p, s).wait()

        @pl.when(p >= 2)
        def _():
            owait(p - 2, s)

        @pl.when(p == 1)
        def _():
            opiece(0, 0, 1, 0, S).start()

        for j in range(2):
            lo = 0
            for n in OSPLIT[j]:
                mm_split(s, j, lo, n, VG, wr_ref)
                opiece(p, s, j, lo, n).start()
                lo += n

        @pl.when(p + 2 < NP)
        def _():
            xcp(p + 2, s).start()

        return c

    lax.fori_loop(1, NP, body, 0)
    owait(NP - 2, (NP - 2) % 2)
    owait(NP - 1, (NP - 1) % 2)


@jax.jit
def pallas_standalone__structured_sparse_n_m__ragged_kernel(
    x: jax.Array,
    w: jax.Array,
    b: jax.Array,
):
    B, S, D = x.shape
    F = GS * len(VG)
    FH = GS * len(HVG)
    KT = D - D // LANES * LANES
    xt = jnp.transpose(x, (0, 2, 1))
    hbm = pl.BlockSpec(memory_space=pltpu.HBM)
    out = pl.pallas_call(
        _kernel,
        in_specs=[hbm, hbm, hbm],
        out_specs=hbm,
        out_shape=jax.ShapeDtypeStruct((B, D, S), x.dtype),
        scratch_shapes=[
            pltpu.VMEM((2, 2, D, S), jnp.bfloat16),
            pltpu.VMEM((2, 2, D, S), jnp.bfloat16),
            pltpu.VMEM((D, D), jnp.bfloat16),
            pltpu.VMEM((D,), jnp.bfloat16),
            pltpu.VMEM((D // 2, D + KA), jnp.uint32),
            pltpu.VMEM((KT // 2, D), jnp.uint32),
            pltpu.VMEM(((D - F) // 2, KT + KA), jnp.uint32),
            pltpu.VMEM(((D - FH) // 2, KT + KA), jnp.uint32),
            pltpu.VMEM((F, LANES), jnp.float32),
            pltpu.VMEM((KT, F, LANES), jnp.float32),
            pltpu.VMEM((F, LANES), jnp.float32),
            pltpu.VMEM((XFS, KT, LANES), jnp.float32),
            pltpu.SemaphoreType.DMA((2,)),
            pltpu.SemaphoreType.DMA((2,)),
            pltpu.SemaphoreType.DMA((2,)),
            pltpu.SemaphoreType.DMA((2 * len(HEAD),)),
        ],
        compiler_params=pltpu.CompilerParams(vmem_limit_bytes=64 << 20),
    )(xt, w, b)
    return jnp.transpose(out, (0, 2, 1))
```
